```python
import jax
import jax.numpy as jnp

def _softmax(x, axis=-1):
    return jax.nn.softmax(x, axis=axis)

def _gelu(x):
    return jax.nn.gelu(x, approximate=True)

def _silu(x):
    return jax.nn.silu(x)

def _sigmoid(x):
    return jax.nn.sigmoid(x)

def _layernorm(x, axis=-1, eps=1e-05):
    m = jnp.mean(x, axis=axis, keepdims=True)
    v = jnp.var(x, axis=axis, keepdims=True)
    return (x - m) / jnp.sqrt(v + eps)

def _scatter_add(tgt, idx, src, axis=0):
    return tgt.at[idx].add(src)

def _segment_sum(src, seg, n):
    return jax.ops.segment_sum(src, seg, n)

class _Rng:

    def __init__(self, key):
        self._k = key

    def _next(self):
        self._k, sub = jax.random.split(self._k)
        return sub

    def normal(self, shape):
        return jax.random.normal(self._next(), shape, dtype=jnp.bfloat16)

    def randint(self, lo, hi, shape):
        return jax.random.randint(self._next(), shape, lo, hi, dtype=jnp.int32)

    def uniform(self, shape, lo=0.0, hi=1.0):
        return jax.random.uniform(self._next(), shape, jnp.bfloat16, lo, hi)

    def permutation(self, n):
        return jax.random.permutation(self._next(), n)
kernel_name = 'adaLN_cond__sliding_block_cached__moe_arch_mod__decode'

def setup_inputs():
    _rng = _Rng(jax.random.key(int.from_bytes(__import__("os").urandom(4), "little")))
    _w = lambda a: (lambda t: t.astype(jnp.bfloat16) if jnp.issubdtype(t.dtype, jnp.floating) else t)(jnp.asarray(a))

    def _A_setup():
        B, Sq, D = (8, 1, 576)
        Hq, Hkv, Sk, Dh = (32, 16, 8192, 128)
        assert Hq % Hkv == 0, (Hq, Hkv)
        return {'x': _w((lambda *s: _rng.normal(s) * 0.05)(B, Sq, D)), 'k_cache': _w((lambda *s: _rng.normal(s) * 0.05)(B, Hkv, Sk, Dh)), 'v_cache': _w((lambda *s: _rng.normal(s) * 0.05)(B, Hkv, Sk, Dh)), 'wq': _w((lambda *s: _rng.normal(s) * 0.05)(D, Hq * Dh) * D ** (-0.5)), 'wo': _w((lambda *s: _rng.normal(s) * 0.05)(Hq * Dh, D) * (Hq * Dh) ** (-0.5))}
    _A_in = _A_setup()

    def _B_setup():
        B, S, D, F, C = (8, 1, 576, 4608, 1)
        return {'x': _w((lambda *s: _rng.normal(s) * 0.05)(B, S, D)), 'w_r': _w((lambda *s: _rng.normal(s) * 0.05)(D)), 'w_gate': _w((lambda *s: _rng.normal(s) * 0.05)(D, F)), 'w_up': _w((lambda *s: _rng.normal(s) * 0.05)(D, F)), 'w_down': _w((lambda *s: _rng.normal(s) * 0.05)(F, D))}
    _B_in = _B_setup()
    return {'A_x': _A_in['x'], 'A_k_cache': _A_in['k_cache'], 'A_v_cache': _A_in['v_cache'], 'A_wq': _A_in['wq'], 'A_wo': _A_in['wo'], 'B_x': _B_in['x'], 'B_w_r': _B_in['w_r'], 'B_w_gate': _B_in['w_gate'], 'B_w_up': _B_in['w_up'], 'B_w_down': _B_in['w_down'], 'c': _w((lambda *s: _rng.normal(s) * 0.05)(8, 576)), 'w_mod': _w((lambda *s: _rng.normal(s) * 0.05)(576, 6 * 576) * 576 ** (-0.5))}

def reference(A_x, A_k_cache, A_v_cache, A_wq, A_wo, B_x, B_w_r, B_w_gate, B_w_up, B_w_down, c, w_mod):

    def _A_ref(x, k_cache, v_cache, wq, wo):
        B, Sq, D = x.shape
        Hq, Dh = (32, 128)
        Hkv, Sk = (k_cache.shape[1], k_cache.shape[2])
        W = min(4096, max(256, Sk // 4))
        rep = Hq // Hkv
        q = (lambda x, *d: x.transpose(*d))((x @ wq).reshape(B, Sq, Hq, Dh), 0, 2, 1, 3)
        k = jnp.repeat(k_cache[:, :, Sk - W:, :], rep, axis=1)
        v = jnp.repeat(v_cache[:, :, Sk - W:, :], rep, axis=1)
        scores = jnp.einsum('bhqd,bhkd->bhqk', q, k) * Dh ** (-0.5)
        p = _softmax(scores, axis=-1)
        o = jnp.einsum('bhqk,bhkd->bhqd', p, v)
        return (lambda x, *d: x.transpose(*d))(o, 0, 2, 1, 3).reshape(B, Sq, Hq * Dh) @ wo

    def _B_ref(x, w_r, w_gate, w_up, w_down):
        B, S, D = x.shape
        C = 1
        r = x @ w_r
        idx = jnp.argsort(-r, axis=-1)[:, :C]
        idx_e = jnp.repeat(idx.reshape(B, C, 1), D, axis=2)
        x_sel = jnp.take_along_axis(x, idx_e, axis=1)
        g = _silu(x_sel @ w_gate)
        u = x_sel @ w_up
        y = g * u @ w_down
        r_sel = _sigmoid(jnp.take_along_axis(r, idx, axis=1))
        y = y * r_sel.reshape(B, C, 1)
        b_off = (jnp.arange(B) * S).reshape(B, 1)
        flat_idx = (idx + b_off).reshape(B * C)
        zero = (x * 0.0).reshape(B * S, D)
        upd = _scatter_add(zero, flat_idx, y.reshape(B * C, D), axis=0)
        return x + upd.reshape(B, S, D)
    x = A_x
    mod = (_silu(c) @ w_mod).reshape(c.shape[0], 6, 1, -1)
    sa, ca, ga, sb, cb, gb = (mod[:, 0].copy(), mod[:, 1].copy(), mod[:, 2].copy(), mod[:, 3].copy(), mod[:, 4].copy(), mod[:, 5].copy())
    h = _layernorm(x, axis=-1) * (1 + ca) + sa
    x = x + ga * _A_ref(h, A_k_cache, A_v_cache, A_wq, A_wo)
    h = _layernorm(x, axis=-1) * (1 + cb) + sb
    x = x + gb * _B_ref(h, B_w_r, B_w_gate, B_w_up, B_w_down)
    return x
```

```python
import functools

import jax
import jax.numpy as jnp
from jax import lax
import jax.experimental.pallas as pl
import jax.experimental.pallas.tpu as pltpu

F32, BF16 = jnp.float32, jnp.bfloat16
NT = (((1,), (1,)), ((), ()))

HQ, DH = 32, 128
SEG = 512
SEG_P0 = 128
LOOK_HEADS = 2
NSLOTS = 4
RB = 16
WLOOK = 16
NSEM = 32


def _layernorm(x):
    m = jnp.mean(x, axis=-1, keepdims=True)
    xc = x - m
    v = jnp.mean(xc * xc, axis=-1, keepdims=True)
    return xc / jnp.sqrt(v + 1e-5)


def _loop(lo, hi, body):
    def f(i, carry):
        body(i)
        return carry

    if hi > lo:
        lax.fori_loop(lo, hi, f, None)


def _kernel(x_hbm, k_hbm, v_hbm, wq_hbm, wo_hbm, wr_hbm, wg_hbm, wu_hbm, wd_hbm, c_hbm, wm_hbm,
            out_ref,
            x_v, c_v, wr_v, wm_v, wq_v, wo_v, wg_v, wu_v, wd_v, kbuf, vbuf, q_s, o_s, sems, ssem):
    B, D = x_hbm.shape
    HKV, SK = k_hbm.shape[1], k_hbm.shape[2]
    W = kbuf.shape[1]
    nseg = W // SEG
    cph = 2 * nseg
    look = LOOK_HEADS * cph
    NWC = D // RB
    NH = B * HKV

    class Weight:
        def __init__(self, hbm, vmem, base):
            self.hbm, self.vmem, self.base = hbm, vmem, base
            self.n = hbm.shape[1]
            self.split = (self.n // 128 // 4) * 128

        def rows(self, i):
            return pl.ds(i * RB if isinstance(i, int) else pl.multiple_of(i * RB, RB), RB)

        def start(self, i, p0=0):
            r = self.rows(i)
            sem = sems.at[(self.base + i) & (NSEM - 1)]
            lo, hi = pl.ds(0, self.split), pl.ds(self.split, self.n - self.split)
            pltpu.make_async_copy(self.hbm.at[r, lo], self.vmem.at[r, lo], sem).start(priority=p0)
            pltpu.make_async_copy(self.hbm.at[r, hi], self.vmem.at[r, hi], sem).start(priority=1)

        def wait(self, i):
            r = self.rows(i)
            sem = sems.at[(self.base + i) & (NSEM - 1)]
            pltpu.make_async_copy(self.vmem.at[r], self.vmem.at[r], sem).wait()

    wm = Weight(wm_hbm, wm_v, 0)
    wq = Weight(wq_hbm, wq_v, NWC)
    kv_base = 2 * NWC
    wo = Weight(wo_hbm, wo_v, kv_base + NH * cph)
    wg = Weight(wg_hbm, wg_v, wo.base + NWC)
    wu = Weight(wu_hbm, wu_v, wg.base + NWC)
    wd = Weight(wd_hbm, wd_v, wu.base + NWC)

    def kv_start(t, s):
        h, b = t // B if isinstance(t, int) else t >> 3, t & (B - 1)
        hbm, buf = (k_hbm, kbuf) if s < nseg else (v_hbm, vbuf)
        sem = sems.at[(kv_base + t * cph + s) & (NSEM - 1)]
        slot = t & (NSLOTS - 1)
        off = (s % nseg) * SEG
        for n, prio in ((SEG_P0, 0), (SEG - SEG_P0, 1)):
            pltpu.make_async_copy(hbm.at[b, h, pl.ds(SK - W + off, n), :],
                                  buf.at[slot, pl.ds(off, n), :], sem).start(priority=prio)
            off += n

    def kv_wait(t, s):
        buf = kbuf if s < nseg else vbuf
        sem = sems.at[(kv_base + t * cph + s) & (NSEM - 1)]
        dst = buf.at[t & (NSLOTS - 1), pl.ds((s % nseg) * SEG, SEG), :]
        pltpu.make_async_copy(dst, dst, sem).wait()

    def stream(cur, nxt):
        def same(i):
            cur.wait(i)
            cur.start(i + WLOOK)

        _loop(0, NWC - WLOOK, same)
        if nxt is not None:
            def cross(i):
                cur.wait(i)
                nxt.start(i - (NWC - WLOOK))

            _loop(NWC - WLOOK, NWC, cross)

    wm.start(0)
    small = [pltpu.make_async_copy(s, d, ssem.at[i])
             for i, (s, d) in enumerate(((c_hbm, c_v), (x_hbm, x_v), (wr_hbm, wr_v)))]
    for cp in small:
        cp.start()
    _loop(1, WLOOK, lambda i: wm.start(i, 1))

    stream(wm, wq)
    for cp in small:
        cp.wait()
    cf = c_v[...].astype(F32)
    sc = (cf * jax.nn.sigmoid(cf)).astype(BF16)
    mod = jnp.dot(sc, wm_v[...], preferred_element_type=F32)
    sa, ca, ga, sb, cb, gb = (mod[:, i * D:(i + 1) * D] for i in range(6))
    x0 = x_v[...].astype(F32)
    h1 = (_layernorm(x0) * (1.0 + ca) + sa).astype(BF16)

    stream(wq, None)
    for j in range(WLOOK):
        wq.wait(NWC - WLOOK + j)
        kv_start(j // cph, j % cph)
    q = jnp.dot(h1, wq_v[...], preferred_element_type=F32)
    for h in range(HKV):
        q_s[h] = jnp.concatenate([q[:, (2 * h) * DH:(2 * h + 1) * DH],
                                  q[:, (2 * h + 1) * DH:(2 * h + 2) * DH]], axis=0).astype(BF16)
    o_s[...] = jnp.zeros(o_s.shape, F32)

    row_b = lax.broadcasted_iota(jnp.int32, (2 * B, DH), 0) & (B - 1)

    def head(t, start_next):
        h, b = t >> 3, t & (B - 1)
        slot = t & (NSLOTS - 1)
        qh = q_s[h]
        ss = []
        for s in range(nseg):
            kv_wait(t, s)
            start_next(s)
            kk = kbuf[slot, pl.ds(s * SEG, SEG), :]
            ss.append(lax.dot_general(qh, kk, NT, preferred_element_type=F32) * (DH ** -0.5))
        m = jnp.max(functools.reduce(jnp.maximum, ss), axis=-1, keepdims=True)
        ps = [jnp.exp(x - m) for x in ss]
        l = jnp.sum(functools.reduce(jnp.add, ps), axis=-1, keepdims=True)
        ps = [p.astype(BF16) for p in ps]
        acc = jnp.zeros((2 * B, DH), F32)
        for s in range(nseg):
            kv_wait(t, nseg + s)
            start_next(nseg + s)
            vv = vbuf[slot, pl.ds(s * SEG, SEG), :]
            acc = acc + jnp.dot(ps[s], vv, preferred_element_type=F32)
        o_s[h] = jnp.where(row_b == b, acc / l, o_s[h])

    _loop(0, NH - LOOK_HEADS, lambda t: head(t, lambda s: kv_start(t + LOOK_HEADS, s)))
    _loop(NH - LOOK_HEADS, NH,
          lambda t: head(t, lambda s: wo.start((t - (NH - LOOK_HEADS)) * cph + s)))

    stream(wo, wg)
    o = jnp.concatenate([o_s[h, pl.ds(r * B, B), :] for h in range(HKV) for r in range(2)], axis=1)
    attn = lax.dot_general(o.astype(BF16), wo_v[...], NT, preferred_element_type=F32)
    x1 = x0 + ga * attn
    h2 = _layernorm(x1) * (1.0 + cb) + sb
    h2b = h2.astype(BF16)
    wr = wr_v[...].astype(F32).reshape(1, D)
    gate = jax.nn.sigmoid(jnp.sum(h2b.astype(F32) * wr, axis=-1, keepdims=True))

    stream(wg, wu)
    g = jnp.dot(h2b, wg_v[...], preferred_element_type=F32)
    g = g * jax.nn.sigmoid(g)
    stream(wu, wd)
    u = jnp.dot(h2b, wu_v[...], preferred_element_type=F32)
    a = (g * u).astype(BF16)

    per = 128 // RB
    for g0 in range(0, NWC, per):
        g1 = min(g0 + per, NWC)

        def step(i):
            wd.wait(i)
            wd.start(i + WLOOK)

        mid = min(max(g0, NWC - WLOOK), g1)
        _loop(g0, mid, step)
        _loop(mid, g1, wd.wait)
        cols = slice(g0 * RB, g1 * RB)
        y = lax.dot_general(a, wd_v[cols, :], NT, preferred_element_type=F32) * gate
        hh = h2[:, cols]
        out_ref[:, cols] = (x1[:, cols] + gb[:, cols] * (hh + (hh * 0.0 + y))).astype(out_ref.dtype)


@jax.jit
def pallas_adaLN_cond__sliding_block_cached__moe_arch_mod__decode_kernel(
    A_x: jax.Array,
    A_k_cache: jax.Array,
    A_v_cache: jax.Array,
    A_wq: jax.Array,
    A_wo: jax.Array,
    B_x: jax.Array,
    B_w_r: jax.Array,
    B_w_gate: jax.Array,
    B_w_up: jax.Array,
    B_w_down: jax.Array,
    c: jax.Array,
    w_mod: jax.Array,
):
    del B_x
    B, S, D = A_x.shape
    HKV, SK = A_k_cache.shape[1], A_k_cache.shape[2]
    W = min(4096, max(256, SK // 4))
    F = B_w_gate.shape[1]
    assert (B, S, HQ // HKV) == (8, 1, 2) and W % SEG == 0 and WLOOK == LOOK_HEADS * 2 * (W // SEG)

    args = (A_x.reshape(B, D), A_k_cache, A_v_cache, A_wq, A_wo.T, B_w_r, B_w_gate, B_w_up,
            B_w_down.T, c, w_mod)
    args = [pltpu.with_memory_space_constraint(a, pltpu.HBM) for a in args]
    out = pl.pallas_call(
        _kernel,
        in_specs=[pl.BlockSpec(memory_space=pltpu.HBM)] * len(args),
        out_specs=pl.BlockSpec(memory_space=pltpu.VMEM),
        out_shape=jax.ShapeDtypeStruct((B, D), A_x.dtype),
        scratch_shapes=[
            pltpu.VMEM((B, D), BF16), pltpu.VMEM((B, D), BF16), pltpu.VMEM((D,), BF16),
            pltpu.VMEM((D, 6 * D), BF16), pltpu.VMEM((D, HQ * DH), BF16), pltpu.VMEM((D, HQ * DH), BF16),
            pltpu.VMEM((D, F), BF16), pltpu.VMEM((D, F), BF16), pltpu.VMEM((D, F), BF16),
            pltpu.VMEM((NSLOTS, W, DH), BF16), pltpu.VMEM((NSLOTS, W, DH), BF16),
            pltpu.VMEM((HKV, 2 * B, DH), BF16), pltpu.VMEM((HKV, 2 * B, DH), F32),
            pltpu.SemaphoreType.DMA((NSEM,)), pltpu.SemaphoreType.DMA((3,)),
        ],
        compiler_params=pltpu.CompilerParams(
            vmem_limit_bytes=100 * 1024 * 1024,
            disable_bounds_checks=True,
            disable_semaphore_checks=True,
        ),
    )(*args)
    return out.reshape(B, S, D)
```

```python
import functools

import jax
import jax.numpy as jnp
from jax import lax
import jax.experimental.pallas as pl
import jax.experimental.pallas.tpu as pltpu

F32, BF16 = jnp.float32, jnp.bfloat16
NT = (((1,), (1,)), ((), ()))

B, D, F = 8, 576, 4608
HQ, HKV, DH = 32, 16, 128
W = 2048
NH = B * HKV
SEG = 512
CW = 512
BAND = 8
NP = 48
NSEM = 32
NSLOTS = 4


def _run(name, lo, sizes):
    out = []
    for n in sizes:
        out.append([(name, lo, n)])
        lo += n
    return out


KV_Q0 = _run("v", 64, [128] * 11)
KV_Q1 = (_run("k", 0, [192] + [256] * 7) + [[("k", 1984, 64), ("v", 0, 64), ("v", 1984, 64)]]
         + _run("v", 1472, [256, 256]))
P = len(KV_Q0)
LOOK = 2 * P
ATTN_AT = (0, 1, 2, 3, 4, 6, 7, 8, 9)
LAST_ROWS = ((0, 256), (384, 576), (256, 384))


def _layernorm(x):
    m = jnp.mean(x, axis=-1, keepdims=True)
    xc = x - m
    v = jnp.mean(xc * xc, axis=-1, keepdims=True)
    return xc / jnp.sqrt(v + 1e-5)


def _silu(x):
    return x * jax.nn.sigmoid(x)


def _loop(lo, hi, body):
    def f(i, carry):
        body(i)
        return carry

    lax.fori_loop(lo, hi, f, None)


def _ds(i, unit, n):
    return pl.ds(i * unit if isinstance(i, int) else pl.multiple_of(i * unit, unit), n)


def _kernel(x_hbm, k_hbm, v_hbm, wq_hbm, wo_hbm, wr_hbm, wg_hbm, wu_hbm, wd_hbm, c_hbm, wm_hbm,
            out_ref,
            x_v, c_v, wr_v, wm_v, wq_v, wo_v, wg_v, wu_v, wd_v, kbuf, vbuf,
            q_s, o_s, mod_s, g_s, a_s, y_s, fin_s, sems, ssem):
    sk = k_hbm.shape[2]

    class Stream:
        def start(self, j, prio=None):
            for src, dst, p in self.copies(j):
                pltpu.make_async_copy(src, dst, self.sem(j)).start(priority=p if prio is None else prio)

        def wait(self, j):
            for src, dst, _ in self.copies(j):
                pltpu.make_async_copy(src, dst, self.sem(j)).wait()

        def sem(self, j):
            return sems.at[(self.base + j) & (NSEM - 1)]

    class Rows(Stream):
        n = NP

        def __init__(self, hbm, vmem, base):
            self.hbm, self.vmem, self.base = hbm, vmem, base

        def copies(self, j):
            n = self.hbm.shape[1]
            half = n // 256 * 128
            if isinstance(j, tuple):
                i, par = j
                cols = pl.ds(0, half) if par == 0 else pl.ds(half, n - half)
                j = 2 * i + par
            else:
                assert 2 * half == n
                i, cols = j >> 1, _ds(j & 1, half, half)
            a, b = (_ds(i, BAND, BAND), cols), (_ds(NP // 2 + j, BAND, BAND), slice(None))
            return [(self.hbm.at[a], self.vmem.at[a], 0), (self.hbm.at[b], self.vmem.at[b], 1)]

        def sem(self, j):
            return super().sem(2 * j[0] + j[1] if isinstance(j, tuple) else j)

    class Cols(Stream):
        full = 8 * (F // CW - 1)

        def __init__(self, hbm, vmem, base):
            self.hbm, self.vmem, self.base = hbm, vmem, base

        def copies(self, j):
            if isinstance(j, int) and j >= self.full:
                r0, r1 = LAST_ROWS[j - self.full]
                a = (pl.ds(r0, r1 - r0), pl.ds(F - CW, CW))
                return [(self.hbm.at[a], self.vmem.at[a], 1)]
            cols, r = _ds(j >> 3, CW, CW), j & 7
            a, b = (_ds(3 * r, BAND, 3 * BAND), cols), (_ds(24 + 6 * r, BAND, 6 * BAND), cols)
            return [(self.hbm.at[a], self.vmem.at[a], 0), (self.hbm.at[b], self.vmem.at[b], 1)]

    class KV(Stream):
        def __init__(self, base):
            self.base = base

        def copies(self, j):
            t, s = j
            h, b, slot = t >> 3, t & (B - 1), t & (NSLOTS - 1)
            out = []
            for prio, parts in ((0, KV_Q0[s]), (1, KV_Q1[s])):
                for name, off, n in parts:
                    hbm, buf = (k_hbm, kbuf) if name == "k" else (v_hbm, vbuf)
                    out.append((hbm.at[b, h, pl.ds(sk - W + off, n), :], buf.at[slot, pl.ds(off, n), :], prio))
            return out

        def sem(self, j):
            return super().sem(j[0] * P + j[1])

    wm = Rows(wm_hbm, wm_v, 0)
    wq = Rows(wq_hbm, wq_v, NP)
    wo = Rows(wo_hbm, wo_v, 2 * NP)
    kv = KV(3 * NP)
    wg = Rows(wg_hbm, wg_v, kv.base + NH * P)
    wu = Rows(wu_hbm, wu_v, wg.base + NP)
    wd = Cols(wd_hbm, wd_v, wu.base + NP)

    def steps(cur, nxt, j0, n):
        def step(r):
            j = j0 + r
            cur.wait(j)
            pl.when(j < NP - LOOK)(lambda: cur.start(j + LOOK))
            pl.when(j >= NP - LOOK)(lambda: nxt.start(j + LOOK - NP))

        _loop(0, n, step)

    wm.start((0, 0))
    small = [pltpu.make_async_copy(s, d, ssem.at[i])
             for i, (s, d) in enumerate(((c_hbm, c_v), (x_hbm, x_v), (wr_hbm, wr_v)))]
    for cp in small:
        cp.start()
    wm.start((0, 1), 1)

    def fill(i):
        wm.start((i, 0), 1)
        wm.start((i, 1), 1)

    _loop(1, LOOK // 2, fill)

    def wm_pair(i):
        for par in range(2):
            wm.wait((i, par))
            pl.when(i < (NP - LOOK) // 2)(lambda: wm.start((i + LOOK // 2, par)))
            pl.when(i >= (NP - LOOK) // 2)(lambda: wq.start(2 * i + par + LOOK - NP))

    _loop(0, NP // 2, wm_pair)
    for cp in small:
        cp.wait()

    sc = _silu(c_v[...].astype(F32)).astype(BF16)

    def mod_piece(i):
        steps(wq, wo, 5 * i, 5)
        cols = _ds(i, 384, 384)
        mod_s[:, cols] = jnp.dot(sc, wm_v[:, cols], preferred_element_type=F32)

    _loop(0, 6 * D // 384, mod_piece)
    sa, ca, ga, sb, cb, gb = (mod_s[:, i * D:(i + 1) * D] for i in range(6))
    x0 = x_v[...].astype(F32)
    h1 = (_layernorm(x0) * (1.0 + ca) + sa).astype(BF16)
    steps(wq, wo, 45, NP - 45)

    o_s[...] = jnp.zeros(o_s.shape, F32)

    def q_piece(i):
        def step(r):
            wo.wait(3 * i + r)
            wo.start(3 * i + r + LOOK)

        _loop(0, 3, step)
        q = jnp.dot(h1, wq_v[:, _ds(i, CW, CW)], preferred_element_type=F32)
        for j in range(2):
            q_s[2 * i + j] = jnp.concatenate(
                [q[:, (2 * j) * DH:(2 * j + 1) * DH], q[:, (2 * j + 1) * DH:(2 * j + 2) * DH]],
                axis=0).astype(BF16)

    _loop(0, HQ * DH // CW, q_piece)
    for j in range(24, NP - LOOK):
        wo.wait(j)
        wo.start(j + LOOK)

    def lead_in(t):
        for s in range(P):
            wo.wait(NP - LOOK + t * P + s)
            kv.start((t, s))

    _loop(0, 2, lead_in)
    for s in range(P):
        kv.wait((0, s))
        kv.start((2, s))

    row_b = lax.broadcasted_iota(jnp.int32, (2 * B, DH), 0) & (B - 1)

    def window(t):
        h, b, slot = (t - 1) >> 3, (t - 1) & (B - 1), (t - 1) & (NSLOTS - 1)
        scores, probs, state = [], [], {}

        def qk(i):
            kk = kbuf[slot, pl.ds(i * SEG, SEG), :]
            scores.append(lax.dot_general(q_s[h], kk, NT, preferred_element_type=F32) * (DH ** -0.5))

        def softmax():
            m = jnp.max(functools.reduce(jnp.maximum, scores), axis=-1, keepdims=True)
            e = [jnp.exp(x - m) for x in scores]
            state["l"] = jnp.sum(functools.reduce(jnp.add, e), axis=-1, keepdims=True)
            probs.extend(x.astype(BF16) for x in e)

        def pv(i):
            r = jnp.dot(probs[i], vbuf[slot, pl.ds(i * SEG, SEG), :], preferred_element_type=F32)
            state["acc"] = r if i == 0 else state["acc"] + r
            if i == W // SEG - 1:
                o_s[h] = jnp.where(row_b == b, state["acc"] / state["l"], o_s[h])

        work = ([functools.partial(qk, i) for i in range(W // SEG)] + [softmax]
                + [functools.partial(pv, i) for i in range(W // SEG)])
        for s in range(P):
            pl.when(t < NH)(lambda: kv.wait((t, s)))
            pl.when(t == NH)(lambda: wg.wait(s))
            pl.when(t < NH - 2)(lambda: kv.start((t + 2, s)))
            pl.when(t >= NH - 2)(lambda: wg.start((t - (NH - 2)) * P + s))
            for w, at in zip(work, ATTN_AT):
                if at == s:
                    w()

    _loop(1, NH + 1, window)

    y_s[...] = jnp.zeros(y_s.shape, F32)

    def wo_piece(i):
        steps(wg, wu, P + 4 * i, 4)
        o = jnp.concatenate([o_s[2 * i + j // 2, pl.ds((j % 2) * B, B), :] for j in range(4)], axis=1)
        y_s[...] += lax.dot_general(o.astype(BF16), wo_v[:, _ds(i, CW, CW)], NT, preferred_element_type=F32)

    _loop(0, HQ * DH // CW, wo_piece)
    x1 = x0 + ga * y_s[...]
    h2 = _layernorm(x1) * (1.0 + cb) + sb
    h2b = h2.astype(BF16)
    wr = wr_v[...].astype(F32).reshape(1, D)
    gate = jax.nn.sigmoid(jnp.sum(h2b.astype(F32) * wr, axis=-1, keepdims=True))
    fin_s[0] = x1 + gb * (h2 + h2 * 0.0)
    fin_s[1] = gb * gate
    steps(wg, wu, P + 32, NP - P - 32)

    def g_piece(i):
        steps(wu, wd, 5 * i, 5)
        cols = _ds(i, CW, CW)
        g_s[:, cols] = _silu(jnp.dot(h2b, wg_v[:, cols], preferred_element_type=F32))

    _loop(0, F // CW, g_piece)
    steps(wu, wd, 45, NP - 45)

    def wd_steps(lo, hi):
        def step(j):
            wd.wait(j)
            pl.when(j + LOOK < wd.full)(lambda: wd.start(j + LOOK))
            for e in range(wd.full, wd.full + len(LAST_ROWS)):
                pl.when(j + LOOK == e)(functools.partial(wd.start, e))

        _loop(lo, hi, step)

    def u_piece(i):
        wd_steps(3 * i, 3 * i + 3)
        cols = _ds(i, CW, CW)
        u = jnp.dot(h2b, wu_v[:, cols], preferred_element_type=F32)
        a_s[:, cols] = (g_s[:, cols] * u).astype(BF16)

    _loop(0, F // CW, u_piece)
    done = 3 * (F // CW)
    y_s[...] = jnp.zeros(y_s.shape, F32)

    def d_piece(i):
        wd_steps(jnp.maximum(8 * i, done), jnp.maximum(8 * i + 8, done))
        cols = _ds(i, CW, CW)
        y_s[...] += lax.dot_general(a_s[:, cols], wd_v[:, cols], NT, preferred_element_type=F32)

    _loop(0, F // CW - 1, d_piece)
    cols = pl.ds(F - CW, CW)
    for e, (r0, r1) in enumerate(LAST_ROWS):
        wd.wait(wd.full + e)
        r = slice(r0, r1)
        y = y_s[:, r] + lax.dot_general(a_s[:, cols], wd_v[r, cols], NT, preferred_element_type=F32)
        out_ref[:, r] = (fin_s[0, :, r] + fin_s[1, :, r] * y).astype(out_ref.dtype)


@jax.jit
def pallas_adaLN_cond__sliding_block_cached__moe_arch_mod__decode_kernel(
    A_x: jax.Array,
    A_k_cache: jax.Array,
    A_v_cache: jax.Array,
    A_wq: jax.Array,
    A_wo: jax.Array,
    B_x: jax.Array,
    B_w_r: jax.Array,
    B_w_gate: jax.Array,
    B_w_up: jax.Array,
    B_w_down: jax.Array,
    c: jax.Array,
    w_mod: jax.Array,
):
    del B_x
    assert A_x.shape == (B, 1, D) and A_k_cache.shape[:2] == (B, HKV) and A_k_cache.shape[3] == DH
    assert min(4096, max(256, A_k_cache.shape[2] // 4)) == W and B_w_gate.shape == (D, F)

    args = (A_x.reshape(B, D), A_k_cache, A_v_cache, A_wq, A_wo.T, B_w_r, B_w_gate, B_w_up,
            B_w_down.T, c, w_mod)
    args = [pltpu.with_memory_space_constraint(a, pltpu.HBM) for a in args]
    out = pl.pallas_call(
        _kernel,
        in_specs=[pl.BlockSpec(memory_space=pltpu.HBM)] * len(args),
        out_specs=pl.BlockSpec(memory_space=pltpu.VMEM),
        out_shape=jax.ShapeDtypeStruct((B, D), A_x.dtype),
        scratch_shapes=[
            pltpu.VMEM((B, D), BF16), pltpu.VMEM((B, D), BF16), pltpu.VMEM((D,), BF16),
            pltpu.VMEM((D, 6 * D), BF16), pltpu.VMEM((D, HQ * DH), BF16), pltpu.VMEM((D, HQ * DH), BF16),
            pltpu.VMEM((D, F), BF16), pltpu.VMEM((D, F), BF16), pltpu.VMEM((D, F), BF16),
            pltpu.VMEM((NSLOTS, W, DH), BF16), pltpu.VMEM((NSLOTS, W, DH), BF16),
            pltpu.VMEM((HKV, 2 * B, DH), BF16), pltpu.VMEM((HKV, 2 * B, DH), F32),
            pltpu.VMEM((B, 6 * D), F32), pltpu.VMEM((B, F), F32), pltpu.VMEM((B, F), BF16),
            pltpu.VMEM((B, D), F32), pltpu.VMEM((2, B, D), F32),
            pltpu.SemaphoreType.DMA((NSEM,)), pltpu.SemaphoreType.DMA((3,)),
        ],
        compiler_params=pltpu.CompilerParams(
            vmem_limit_bytes=64 * 1024 * 1024,
            disable_bounds_checks=True,
            disable_semaphore_checks=True,
        ),
    )(*args)
    return out.reshape(B, 1, D)
```

```python
import functools

import jax
import jax.numpy as jnp
from jax import lax
import jax.experimental.pallas as pl
import jax.experimental.pallas.tpu as pltpu

F32, BF16 = jnp.float32, jnp.bfloat16
NT = (((1,), (1,)), ((), ()))

B, D, F = 8, 576, 4608
HQ, HKV, DH = 32, 16, 128
W = 2048
G = 8
NG = B * HKV // G
ROWS = 64
PK = W // ROWS
KP = 512
SUB = 9
SR = D // SUB
BAND = 8
CW = 512
LOOK = 16
NSEM = 32
DOWN_RUNS = (4, 2, 1, 1)
LAST_ROWS = ((0, 256), (384, 576), (256, 384))


def _layernorm(x):
    m = jnp.mean(x, axis=-1, keepdims=True)
    xc = x - m
    v = jnp.mean(xc * xc, axis=-1, keepdims=True)
    return xc / jnp.sqrt(v + 1e-5)


def _silu(x):
    return x * jax.nn.sigmoid(x)


def _loop(lo, hi, body):
    def f(i, carry):
        body(i)
        return carry

    lax.fori_loop(lo, hi, f, None)


def _div(j, n):
    if n & (n - 1) == 0:
        return j >> (n.bit_length() - 1)
    return (j * (-(-65536 // n))) >> 16


def _ds(i, n):
    return pl.ds(i * n if isinstance(i, int) else pl.multiple_of(i * n, n), n)


def _kernel(x_hbm, k_hbm, v_hbm, wq_hbm, wo_hbm, wr_hbm, wg_hbm, wu_hbm, wd_hbm, c_hbm, wm_hbm,
            out_ref,
            x_v, c_v, wr_v, wm_v, wq_v, wo_v, wg_v, wu_v, wd_v, kbuf, vbuf,
            q_s, s_s, p_s, l_s, o_s, mod_s, g_s, a_s, y_s, fin_s, sems, ssem):
    sk = k_hbm.shape[2]

    class Stream:
        def start(self, j, prio=None):
            for src, dst, p in self.copies(j):
                pltpu.make_async_copy(src, dst, self.sem(j)).start(priority=p if prio is None else prio)

        def wait(self, j):
            for src, dst, _ in self.copies(j):
                pltpu.make_async_copy(src, dst, self.sem(j)).wait()

        def sem(self, j):
            return sems.at[(self.base + j) & (NSEM - 1)]

    class Weight(Stream):
        def __init__(self, hbm, vmem, base, cw=CW, c0=0, nc=None):
            self.hbm, self.vmem, self.base, self.cw, self.c0 = hbm, vmem, base, cw, c0
            self.nc = nc or hbm.shape[2] // cw
            self.n = self.nc * (SR // BAND)

        def copies(self, j):
            band = _div(j, self.nc)
            r, c = _ds(band, BAND), _ds(self.c0 + j - band * self.nc, self.cw)
            return [(self.hbm.at[blocks, r, c], self.vmem.at[blocks, r, c], p)
                    for blocks, p in ((pl.ds(0, 1), 0), (pl.ds(1, SUB - 1), 1))]

    class LastRows(Stream):
        n = len(LAST_ROWS)

        def __init__(self, base):
            self.base = base

        def copies(self, j):
            r0, r1 = LAST_ROWS[j]
            idx = (pl.ds(r0 // SR, (r1 - r0) // SR), slice(None), pl.ds(F - CW, CW))
            return [(wd_hbm.at[idx], wd_v.at[idx], 1)]

    class Cache(Stream):
        n = PK

        def __init__(self, hbm, buf, g, base):
            self.hbm, self.buf, self.g, self.base = hbm, buf, g, base

        def copies(self, j):
            b, h0 = self.g >> 1, (self.g & 1) * G
            src, dst = _ds((sk - W) // ROWS + j, ROWS), _ds(j, ROWS)
            return [(self.hbm.at[b, pl.ds(h0 + lo, n), src, :],
                     self.buf.at[self.g & 1, pl.ds(lo, n), dst, :], p)
                    for lo, n, p in ((0, 1, 0), (1, G - 1, 1))]

    wm = Weight(wm_hbm, wm_v, 0, cw=384)
    wq = Weight(wq_hbm, wq_v, wm.n)
    kv0 = wm.n + wq.n
    keys = lambda g: Cache(k_hbm, kbuf, g, kv0 + 2 * PK * g)
    vals = lambda g: Cache(v_hbm, vbuf, g, kv0 + 2 * PK * g + PK)
    wo = Weight(wo_hbm, wo_v, kv0 + 2 * PK * NG)
    wg = Weight(wg_hbm, wg_v, wo.base + wo.n)
    wu = Weight(wu_hbm, wu_v, wg.base + wg.n)
    wds, base, c0 = [], wu.base + wu.n, 0
    for nc in DOWN_RUNS:
        wds.append(Weight(wd_hbm, wd_v, base, c0=c0, nc=nc))
        base, c0 = base + wds[-1].n, c0 + nc
    wds.append(LastRows(base))

    def steps(lo, hi, cur, nxt):
        def step(j):
            cur.wait(j)
            t = j + LOOK
            pl.when(t < cur.n)(lambda: cur.start(t))
            pl.when(t >= cur.n)(lambda: nxt.start(t - cur.n))

        _loop(lo, hi, step)

    def weight(ref, cols):
        w = ref[:, :, cols]
        return w.reshape(D, w.shape[-1])

    wm.start(0)
    small = [pltpu.make_async_copy(s, d, ssem.at[i])
             for i, (s, d) in enumerate(((c_hbm, c_v), (x_hbm, x_v), (wr_hbm, wr_v)))]
    for cp in small:
        cp.start()
    _loop(1, LOOK, wm.start)
    steps(0, wm.n, wm, wq)
    for cp in small:
        cp.wait()

    sc = _silu(c_v[...].astype(F32)).astype(BF16)

    def mod_piece(i):
        steps(6 * i, 6 * i + 6, wq, keys(0))
        cols = _ds(i, wm.cw)
        mod_s[:, cols] = jnp.dot(sc, weight(wm_v, cols), preferred_element_type=F32)

    _loop(0, wm.nc, mod_piece)
    sa, ca, ga, sb, cb, gb = (mod_s[:, i * D:(i + 1) * D] for i in range(6))
    x0 = x_v[...].astype(F32)
    h1 = (_layernorm(x0) * (1.0 + ca) + sa).astype(BF16)
    steps(6 * wm.nc, wq.n, wq, keys(0))

    s_s[...] = jnp.zeros(s_s.shape, F32)
    o_s[...] = jnp.zeros(o_s.shape, F32)

    def q_piece(i):
        per = PK // wq.nc
        steps(i * per, (i + 1) * per, keys(0), vals(0))
        q = jnp.dot(h1, weight(wq_v, _ds(i, CW)), preferred_element_type=F32)
        for j in range(CW // DH):
            q_s[pl.ds(i * (CW // DH) + j, B, stride=HQ), :] = q[:, j * DH:(j + 1) * DH]

    _loop(0, wq.nc, q_piece)

    def group(g):
        v, nk, nv = vals(g), keys(g + 1), vals(g + 1)
        more = g < NG - 1
        heads = _ds(g, 2 * G)

        def qk_piece(i):
            def step(j):
                v.wait(j)
                t = j + LOOK
                pl.when(t < PK)(lambda: v.start(t))
                pl.when((t >= PK) & more)(lambda: nk.start(t - PK))
                pl.when((t >= PK) & jnp.logical_not(more))(lambda: wo.start(t - PK))

            per = PK * KP // (G * W)
            _loop(i * per, (i + 1) * per, step)
            h, cols = _div(i, W // KP), _ds(i & (W // KP - 1), KP)
            s = lax.dot_general(q_s[heads, :].astype(BF16), kbuf[g & 1, h, cols, :], NT,
                                preferred_element_type=F32)
            mine = lax.broadcasted_iota(jnp.int32, s.shape, 0) >> 1 == h
            s_s[:, cols] = jnp.where(mine, s, s_s[:, cols])

        _loop(0, G * W // KP, qk_piece)
        s = s_s[...] * (DH ** -0.5)
        e = jnp.exp(s - jnp.max(s, axis=-1, keepdims=True))
        l_s[...] = jnp.broadcast_to(jnp.sum(e, axis=-1, keepdims=True), l_s.shape)
        p_s[...] = e.astype(BF16)

        def pv_piece(h):
            def step(j):
                t = j + LOOK

                @pl.when(more)
                def _():
                    nk.wait(j)
                    pl.when(t < PK)(lambda: nk.start(t))
                    pl.when(t >= PK)(lambda: nv.start(t - PK))

                @pl.when(jnp.logical_not(more))
                def _():
                    wo.wait(j)
                    wo.start(t)

            per = PK // G
            _loop(h * per, (h + 1) * per, step)
            o = jnp.dot(p_s[...], vbuf[g & 1, h], preferred_element_type=F32) / l_s[...]
            mine = lax.broadcasted_iota(jnp.int32, o.shape, 0) >> 1 == h
            o_s[heads, :] = jnp.where(mine, o, o_s[heads, :])

        _loop(0, G, pv_piece)

    _loop(0, NG, group)
    steps(PK, wo.n, wo, wg)

    y_s[...] = jnp.zeros(y_s.shape, F32)

    def wo_piece(i):
        steps(6 * i, 6 * i + 6, wg, wu)
        o = jnp.concatenate(
            [o_s[pl.ds(i * (CW // DH) + j, B, stride=HQ), :] for j in range(CW // DH)], axis=1)
        y_s[...] += lax.dot_general(o.astype(BF16), weight(wo_v, _ds(i, CW)), NT,
                                    preferred_element_type=F32)

    _loop(0, wo.nc, wo_piece)
    x1 = x0 + ga * y_s[...]
    h2 = _layernorm(x1) * (1.0 + cb) + sb
    h2b = h2.astype(BF16)
    wr = wr_v[...].astype(F32).reshape(1, D)
    gate = jax.nn.sigmoid(jnp.sum(h2b.astype(F32) * wr, axis=-1, keepdims=True))
    fin_s[0] = x1 + gb * (h2 + h2 * 0.0)
    fin_s[1] = gb * gate
    steps(6 * wo.nc, wg.n, wg, wu)

    def gate_piece(i):
        steps(8 * i, 8 * i + 8, wu, wds[0])
        cols = _ds(i, CW)
        g_s[:, cols] = _silu(jnp.dot(h2b, weight(wg_v, cols), preferred_element_type=F32))

    _loop(0, wg.nc, gate_piece)

    def up(i):
        cols = _ds(i, CW)
        u = jnp.dot(h2b, weight(wu_v, cols), preferred_element_type=F32)
        a_s[:, cols] = (g_s[:, cols] * u).astype(BF16)

    def down(i):
        cols = _ds(i, CW)
        y_s[...] += lax.dot_general(a_s[:, cols], weight(wd_v, cols), NT, preferred_element_type=F32)

    y_s[...] = jnp.zeros(y_s.shape, F32)
    periods = [(w, j) for w in wds for j in range(w.n)]
    landed = [sum(w.n for w in wds[:n + 1]) for n in range(len(DOWN_RUNS)) for _ in range(wds[n].nc)]
    work = [(0, 3, functools.partial(up, i)) for i in range(F // CW)]
    work += [(at, 4, functools.partial(down, i)) for i, at in enumerate(landed)]
    free = 1
    for n in range(landed[-1]):
        periods[n][0].wait(periods[n][1])
        if n + LOOK < len(periods):
            periods[n + LOOK][0].start(periods[n + LOOK][1])
        if work and n + 1 >= max(free, work[0][0]):
            _, gap, f = work.pop(0)
            f()
            free = n + 1 + gap
    for _, _, f in work:
        f()
    cols = pl.ds(F - CW, CW)
    for e, (r0, r1) in enumerate(LAST_ROWS):
        wds[-1].wait(e)
        r = slice(r0, r1)
        w = wd_v[r0 // SR:r1 // SR, :, cols].reshape(r1 - r0, CW)
        y = y_s[:, r] + lax.dot_general(a_s[:, cols], w, NT, preferred_element_type=F32)
        out_ref[:, r] = (fin_s[0, :, r] + fin_s[1, :, r] * y).astype(out_ref.dtype)


@jax.jit
def pallas_adaLN_cond__sliding_block_cached__moe_arch_mod__decode_kernel(
    A_x: jax.Array,
    A_k_cache: jax.Array,
    A_v_cache: jax.Array,
    A_wq: jax.Array,
    A_wo: jax.Array,
    B_x: jax.Array,
    B_w_r: jax.Array,
    B_w_gate: jax.Array,
    B_w_up: jax.Array,
    B_w_down: jax.Array,
    c: jax.Array,
    w_mod: jax.Array,
):
    del B_x
    assert A_x.shape == (B, 1, D) and B_w_gate.shape == (D, F)
    assert A_k_cache.shape == (B, HKV, 4 * W, DH) and A_wq.shape == (D, HQ * DH)

    blocks = lambda w: w.reshape(SUB, SR, w.shape[1])
    args = (A_x.reshape(B, D), A_k_cache, A_v_cache, blocks(A_wq), blocks(A_wo.T), B_w_r,
            blocks(B_w_gate), blocks(B_w_up), blocks(B_w_down.T), c, blocks(w_mod))
    wbuf = lambda n: pltpu.VMEM((SUB, SR, n), BF16)
    out = pl.pallas_call(
        _kernel,
        in_specs=[pl.BlockSpec(memory_space=pltpu.HBM)] * len(args),
        out_specs=pl.BlockSpec(memory_space=pltpu.VMEM),
        out_shape=jax.ShapeDtypeStruct((B, D), A_x.dtype),
        scratch_shapes=[
            pltpu.VMEM((B, D), BF16), pltpu.VMEM((B, D), BF16), pltpu.VMEM((D,), BF16),
            wbuf(6 * D), wbuf(HQ * DH), wbuf(HQ * DH), wbuf(F), wbuf(F), wbuf(F),
            pltpu.VMEM((2, G, W, DH), BF16), pltpu.VMEM((2, G, W, DH), BF16),
            pltpu.VMEM((B * HQ, DH), F32), pltpu.VMEM((2 * G, W), F32), pltpu.VMEM((2 * G, W), BF16),
            pltpu.VMEM((2 * G, DH), F32), pltpu.VMEM((B * HQ, DH), F32),
            pltpu.VMEM((B, 6 * D), F32), pltpu.VMEM((B, F), F32), pltpu.VMEM((B, F), BF16),
            pltpu.VMEM((B, D), F32), pltpu.VMEM((2, B, D), F32),
            pltpu.SemaphoreType.DMA((NSEM,)), pltpu.SemaphoreType.DMA((3,)),
        ],
        compiler_params=pltpu.CompilerParams(
            vmem_limit_bytes=120 * 1024 * 1024,
            disable_bounds_checks=True,
            disable_semaphore_checks=True,
        ),
    )(*args)
    return out.reshape(B, 1, D)
```
